```python
import os as _os
_os.environ.setdefault("JAX_PLATFORMS", "cpu")
import jax
import jax.numpy as jnp

def _softmax(x, axis=-1):
    return jax.nn.softmax(x, axis=axis)
def _gelu(x):
    return jax.nn.gelu(x, approximate=True)
def _silu(x):
    return jax.nn.silu(x)
def _sigmoid(x):
    return jax.nn.sigmoid(x)
def _layernorm(x, axis=-1, eps=1e-5):
    m = jnp.mean(x, axis=axis, keepdims=True)
    v = jnp.var(x, axis=axis, keepdims=True)
    return (x - m) / jnp.sqrt(v + eps)
def _scatter_add(tgt, idx, src, axis=0):
    return tgt.at[idx].add(src)
def _segment_sum(src, seg, n):
    return jax.ops.segment_sum(src, seg, n)
class _Rng:
    def __init__(self, key):
        self._k = key
    def _next(self):
        self._k, sub = jax.random.split(self._k)
        return sub
    def normal(self, shape):
        return jax.random.normal(self._next(), shape, dtype=jnp.bfloat16)
    def randint(self, lo, hi, shape):
        return jax.random.randint(self._next(), shape, lo, hi, dtype=jnp.int32)
    def uniform(self, shape, lo=0.0, hi=1.0):
        return jax.random.uniform(self._next(), shape, jnp.bfloat16, lo, hi)
    def permutation(self, n):
        return jax.random.permutation(self._next(), n)


kernel_name = 'concat_heads__mha_block_cached__gqa_block_cached__near_ridge'

def setup_inputs():
    _rng = _Rng(jax.random.key(int.from_bytes(__import__("os").urandom(4), "little")))
    _w = (lambda a: (lambda t: t.astype(jnp.bfloat16) if jnp.issubdtype(t.dtype, jnp.floating) else t)(jnp.asarray(a)))
    def _A_setup():
        B, Sq, D = 16, 160, 512
        H, Sk, Dh = 32, 1024, 128
        return {
            "x": _w((lambda *s: _rng.normal(s) * 0.8)(B, Sq, D)),
            "k_cache": _w((lambda *s: _rng.normal(s) * 0.8)(B, H, Sk, Dh)),
            "v_cache": _w((lambda *s: _rng.normal(s) * 0.05)(B, H, Sk, Dh)),
            "wq": _w((lambda *s: _rng.normal(s) * 0.8)(D, H * Dh) * (D ** -0.5)),
            "wo": _w((lambda *s: _rng.normal(s) * 0.05)(H * Dh, D) * ((H * Dh) ** -0.5)),
        }
    _A_in = _A_setup()

    def _B_setup():
        B, Sq, D = 16, 160, 512
        Hq, Hkv, Sk, Dh = 32, 32, 1024, 128
        assert Hq % Hkv == 0, (Hq, Hkv)
        return {
            "x": _w((lambda *s: _rng.normal(s) * 0.8)(B, Sq, D)),
            "k_cache": _w((lambda *s: _rng.normal(s) * 0.8)(B, Hkv, Sk, Dh)),
            "v_cache": _w((lambda *s: _rng.normal(s) * 0.05)(B, Hkv, Sk, Dh)),
            "wq": _w((lambda *s: _rng.normal(s) * 0.8)(D, Hq * Dh) * (D ** -0.5)),
            "wo": _w((lambda *s: _rng.normal(s) * 0.05)(Hq * Dh, D) * ((Hq * Dh) ** -0.5)),
        }
    _B_in = _B_setup()

    return {
        "A_x": _A_in["x"],
        "A_k_cache": _A_in["k_cache"],
        "A_v_cache": _A_in["v_cache"],
        "A_wq": _A_in["wq"],
        "A_wo": _A_in["wo"],
        "B_x": _B_in["x"],
        "B_k_cache": _B_in["k_cache"],
        "B_v_cache": _B_in["v_cache"],
        "B_wq": _B_in["wq"],
        "B_wo": _B_in["wo"],
    }

def reference(A_x, A_k_cache, A_v_cache, A_wq, A_wo, B_x, B_k_cache, B_v_cache, B_wq, B_wo):
    def _A_ref(x, k_cache, v_cache, wq, wo):
        B, Sq, D = x.shape
        H, Dh = 32, 128
        q = (lambda x, *d: x.transpose(*d))((x @ wq).reshape(B, Sq, H, Dh), 0, 2, 1, 3)
        scores = jnp.einsum("bhqd,bhkd->bhqk", q, k_cache) * (Dh ** -0.5)
        p = _softmax(scores, axis=-1)
        o = jnp.einsum("bhqk,bhkd->bhqd", p, v_cache)
        return (lambda x, *d: x.transpose(*d))(o, 0, 2, 1, 3).reshape(B, Sq, H * Dh) @ wo

    def _B_ref(x, k_cache, v_cache, wq, wo):
        B, Sq, D = x.shape
        Hq, Dh = 32, 128
        Hkv = k_cache.shape[1]
        rep = Hq // Hkv
        q = (lambda x, *d: x.transpose(*d))((x @ wq).reshape(B, Sq, Hq, Dh), 0, 2, 1, 3)
        k = jnp.repeat(k_cache, rep, axis=1)
        v = jnp.repeat(v_cache, rep, axis=1)
        scores = jnp.einsum("bhqd,bhkd->bhqk", q, k) * (Dh ** -0.5)
        p = _softmax(scores, axis=-1)
        o = jnp.einsum("bhqk,bhkd->bhqd", p, v)
        return (lambda x, *d: x.transpose(*d))(o, 0, 2, 1, 3).reshape(B, Sq, Hq * Dh) @ wo

    a = _A_ref(A_x, A_k_cache, A_v_cache, A_wq, A_wo)
    b = _B_ref(B_x, B_k_cache, B_v_cache, B_wq, B_wo)
    return jnp.concatenate([a, b], axis=-1)
```

```python
import math

import jax
import jax.numpy as jnp
from jax import lax
import jax.experimental.pallas as pl
import jax.experimental.pallas.tpu as pltpu

DH = 128
G = 4
DIST = 2
NSLOT = DIST + 2
KV_ROWS = 128
X_ROWS = 32
_NT = (((1,), (1,)), ((), ()))


def _make_kernel(B, SQ, D, H, SK):
    bf16, f32 = jnp.bfloat16, jnp.float32
    assert B & (B - 1) == 0 and B > DIST + 1 and H % G == 0 and H > G
    log_b = B.bit_length() - 1
    nstep = B * (H // G)
    nh = 2 * G
    gw = G * DH
    wq_rows, wo_rows = D // B, gw // B
    qscale = DH**-0.5 * math.log2(math.e)
    nchunk = SK // KV_ROWS
    kv_order = [
        (j, h * SK + (c + 4 * h + j) % nchunk * KV_ROWS)
        for c in range(nchunk)
        for h in range(G)
        for j in range(4)
    ]
    step_items = [
        item
        for n in range(nh)
        for item in (("qk", n), ("qp", n + 1), ("pv", n - 1), ("op", n - 2))
    ]

    def kernel(
        ax, ak, av, awq, awo, bx, bk, bv, bwq, bwo, out,
        xs, wq, wo, kv, acc, ob, q_carry, p_carry, r_carry, o_carry,
        pro_sem, kv_sem, w_sem, x_sem, o_sem,
    ):
        caches = (ak, av, bk, bv)

        def start_all(copies):
            for n, cp in enumerate(copies):
                cp.start(priority=n % 2)

        def kv_copies(i, slot, lo, hi):
            base = ((i & (B - 1)) * H + (i >> log_b) * G) * SK
            return [
                pltpu.make_async_copy(
                    caches[j].at[pl.ds(pl.multiple_of(base + r, KV_ROWS), KV_ROWS)],
                    kv.at[slot, j, pl.ds(r, KV_ROWS)],
                    kv_sem.at[slot],
                )
                for j, r in kv_order[lo:hi]
            ]

        def w_copies(w, sem):
            col = pl.multiple_of((w >> log_b) * gw, gw)
            rq = pl.ds(pl.multiple_of((w & (B - 1)) * wq_rows, wq_rows), wq_rows)
            ro = pl.ds(pl.multiple_of(col + (w & (B - 1)) * wo_rows, wo_rows), wo_rows)
            cols = pl.ds(col, gw)
            return [
                pltpu.make_async_copy(awq.at[rq, cols], wq.at[0, rq, cols], sem),
                pltpu.make_async_copy(awo.at[ro], wo.at[0, ro], sem),
                pltpu.make_async_copy(bwq.at[rq, cols], wq.at[1, rq, cols], sem),
                pltpu.make_async_copy(bwo.at[ro], wo.at[1, ro], sem),
            ]

        def x_copies(b, sem):
            return [
                pltpu.make_async_copy(
                    x.at[b, pl.ds(r, X_ROWS)], xs.at[b, br, pl.ds(r, X_ROWS)], sem
                )
                for r in range(0, SQ, X_ROWS)
                for br, x in enumerate((ax, bx))
            ]

        def o_copy(b):
            return pltpu.make_async_copy(ob.at[b], out.at[b], o_sem.at[0])

        def load_kv(slot, j, h):
            words = kv.bitcast(jnp.uint32)[slot, j, pl.ds(h * SK // 2, SK // 2)]
            return pltpu.bitcast(words, bf16)

        def run(i, slot, items, hook=None):
            qs, ps, os_ = {}, {}, {}
            prev_slot = jnp.where(slot == 0, NSLOT - 1, slot - 1)
            for t, (stage, n) in enumerate(items):
                if hook is not None:
                    hook(t)
                step = i + n // nh
                if n < 0:
                    step = jnp.maximum(step, 0)
                if n >= nh:
                    step = jnp.minimum(step, nstep - 1)
                b = step & (B - 1)
                br, h = divmod(n % nh, G)
                head = pl.ds(pl.multiple_of(((step >> log_b) * G + h) * DH, DH), DH)
                if stage == "qp":
                    q = jnp.dot(xs[b, br], wq[br, :, head], preferred_element_type=f32)
                    q = (q * qscale).astype(bf16)
                    if ("qk", n) in items:
                        qs[n] = q
                    else:
                        q_carry[...] = q
                elif stage == "qk":
                    q = qs.pop(n) if n in qs else q_carry[...]
                    s = lax.dot_general(
                        q, load_kv(slot, 2 * br, h), _NT, preferred_element_type=f32
                    )
                    p = jnp.exp2(s - jnp.max(s, axis=-1, keepdims=True))
                    l = jnp.sum(p, axis=-1, keepdims=True)
                    r = pl.reciprocal(l, approx=True)
                    r = r * (2.0 - l * r)
                    p = p.astype(bf16)
                    if ("pv", n) in items:
                        ps[n] = (p, r)
                    else:
                        p_carry[...] = p
                        r_carry[...] = jnp.broadcast_to(r, (SQ, DH))
                elif stage == "pv":
                    p, r = ps.pop(n) if n in ps else (p_carry[...], r_carry[...])
                    v = load_kv(slot if n >= 0 else prev_slot, 2 * br + 1, h)
                    o = jnp.dot(p, v, preferred_element_type=f32)
                    o = (o * r).astype(bf16)
                    if ("op", n) in items:
                        os_[n] = o
                    else:
                        o_carry[...] = o
                else:
                    o = os_.pop(n) if n in os_ else o_carry[...]
                    if n < 0:
                        b = jnp.where(i == 0, B, b)
                    a = acc[b, br] + jnp.dot(
                        o, wo[br, head, :], preferred_element_type=f32
                    )
                    acc[b, br] = a
                    if h == G - 1:
                        ob[b, :, br * D : (br + 1) * D] = a.astype(bf16)

        first = x_copies(0, pro_sem.at[0])
        for w in range(B):
            first += w_copies(w, pro_sem.at[0])
        start_all(first)
        acc[...] = jnp.zeros_like(acc)
        o_carry[...] = jnp.zeros_like(o_carry)
        p_carry[...] = jnp.zeros_like(p_carry)
        r_carry[...] = jnp.zeros_like(r_carry)
        kv[NSLOT - 1, 3, pl.ds((G - 1) * SK, SK)] = jnp.zeros((SK, DH), bf16)
        for s in range(DIST):
            start_all(x_copies(s + 1, x_sem.at[s]) + w_copies(s + B, w_sem.at[s]))
            start_all(kv_copies(s, s, 0, len(kv_order)))
        for cp in first:
            cp.wait()
        run(0, 0, [("qp", 0)])

        def step_body(i, slot):
            pltpu.make_async_copy(kv.at[slot], kv.at[slot], kv_sem.at[slot]).wait()

            @pl.when(i + B < nstep)
            def _():
                for cp in w_copies(i + B, w_sem.at[slot]):
                    cp.wait()

            @pl.when(i + 1 < B)
            def _():
                pltpu.make_async_copy(xs.at[i + 1], xs.at[i + 1], x_sem.at[slot]).wait()

            nxt = slot + DIST
            nxt = jnp.where(nxt >= NSLOT, nxt - NSLOT, nxt)
            per_item = len(kv_order) // len(step_items)

            def issue(t):
                if t == 1:

                    @pl.when(i + DIST + B < nstep)
                    def _():
                        start_all(w_copies(i + DIST + B, w_sem.at[nxt]))

                if t == 2:

                    @pl.when(i + DIST + 1 < B)
                    def _():
                        start_all(x_copies(i + DIST + 1, x_sem.at[nxt]))

                @pl.when(i + DIST < nstep)
                def _():
                    start_all(kv_copies(i + DIST, nxt, t * per_item, (t + 1) * per_item))

                if t % 2 == 0 and t // 2 < B - DIST - 1:

                    @pl.when(i == nstep - DIST)
                    def _():
                        o_copy(t // 2).start()

                if t == 3:

                    @pl.when(i > nstep - DIST)
                    def _():
                        o_copy(i - (nstep - B) - 2).start()

            run(i, slot, step_items, issue)
            return jnp.where(slot == NSLOT - 1, 0, slot + 1)

        lax.fori_loop(0, nstep, step_body, 0)
        o_copy(B - 2).start()
        run(nstep, nstep % NSLOT, [("pv", -1), ("op", -2), ("op", -1)])
        o_copy(B - 1).start()
        pltpu.make_async_copy(ob.at[pl.ds(0, B)], out, o_sem.at[0]).wait()

    assert len(kv_order) % (2 * len(step_items)) == 0
    assert 2 * (B - DIST - 1) <= len(step_items)
    dma_sem = pltpu.SemaphoreType.DMA
    scratch = [
        pltpu.VMEM((B, 2, SQ, D), bf16),
        pltpu.VMEM((2, D, H * DH), bf16),
        pltpu.VMEM((2, H * DH, D), bf16),
        pltpu.VMEM((NSLOT, 4, G * SK, DH), bf16),
        pltpu.VMEM((B + 1, 2, SQ, D), f32),
        pltpu.VMEM((B + 1, SQ, 2 * D), bf16),
        pltpu.VMEM((SQ, DH), bf16),
        pltpu.VMEM((SQ, SK), bf16),
        pltpu.VMEM((SQ, DH), f32),
        pltpu.VMEM((SQ, DH), bf16),
        dma_sem((1,)),
        dma_sem((NSLOT,)),
        dma_sem((NSLOT,)),
        dma_sem((NSLOT,)),
        dma_sem((1,)),
    ]
    return kernel, scratch


@jax.jit
def pallas_concat_heads__mha_block_cached__gqa_block_cached__near_ridge_kernel(
    A_x: jax.Array,
    A_k_cache: jax.Array,
    A_v_cache: jax.Array,
    A_wq: jax.Array,
    A_wo: jax.Array,
    B_x: jax.Array,
    B_k_cache: jax.Array,
    B_v_cache: jax.Array,
    B_wq: jax.Array,
    B_wo: jax.Array,
):
    B, SQ, D = A_x.shape
    _, H, SK, dh = A_k_cache.shape
    assert dh == DH and B_x.shape == A_x.shape and B_k_cache.shape == A_k_cache.shape
    kernel, scratch = _make_kernel(B, SQ, D, H, SK)

    def rows(cache):
        return cache.reshape(B * H * SK, DH)

    return pl.pallas_call(
        kernel,
        in_specs=[pl.BlockSpec(memory_space=pl.ANY)] * 10,
        out_specs=pl.BlockSpec(memory_space=pl.ANY),
        out_shape=jax.ShapeDtypeStruct((B, SQ, 2 * D), A_x.dtype),
        scratch_shapes=scratch,
        compiler_params=pltpu.CompilerParams(
            vmem_limit_bytes=100 * 1024 * 1024, disable_bounds_checks=True
        ),
    )(
        A_x, rows(A_k_cache), rows(A_v_cache), A_wq, A_wo,
        B_x, rows(B_k_cache), rows(B_v_cache), B_wq, B_wo,
    )
```

```python
import math

import jax
import jax.numpy as jnp
from jax import lax
import jax.experimental.pallas as pl
import jax.experimental.pallas.tpu as pltpu

DH = 128
G = 4
NSLOT = 4
KV_ROWS = 128
LEAD = (22, 48)
Q_AHEAD = 4
WQ_SPLIT = 4
OUT_ROWS = 8
SOFTMAX_ROWS = 16

STEP_ITEMS = (
    ("pv", -1), ("op", -3), ("op", -2), ("qk", 0), ("qp", 0), ("qk", 1), ("qp", 1), ("pv", 0),
    ("qk", 2), ("qp", 2), ("pv", 1), ("op", -1), ("op", 0), ("qk", 3), ("qp", 3), ("pv", 2),
    ("qk", 4), ("op", 1), ("qp", 4), ("op", 2), ("pv", 3), ("qk", 5), ("qp", 5), ("pv", 4),
    ("op", 3), ("qk", 6), ("qp", 6), ("qk", 7), ("pv", 5), ("op", 4), ("qp", 7), ("pv", 6),
)
DRAIN_ITEMS = (("pv", -1), ("op", -3), ("op", -2), ("op", -1))
_NT = (((1,), (1,)), ((), ()))


def _scattered_pairs(n):
    npairs = n // 2
    assert n % 2 == 0 and math.gcd(9, npairs) == 1
    return [(2 * (9 * k % npairs) + 1 + u) % n for k in range(npairs) for u in range(2)]


def _kv_orders(sk):
    nchunk = G * sk // KV_ROWS
    nblock = 2 * nchunk
    assert math.gcd(9, nblock) == 1
    orders = ([], [])
    for k in range(nblock):
        pair, cache = divmod(9 * k % nblock, 4)
        for u in range(2):
            orders[k % 2].append((cache, (2 * pair + 1 + u) % nchunk * KV_ROWS))
    shift = LEAD[1] - LEAD[0]
    return orders[0][shift:] + orders[0][:shift], orders[1]


def _make_kernel(B, SQ, D, H, SK):
    bf16, f32 = jnp.bfloat16, jnp.float32
    log_b = B.bit_length() - 1
    nstep = B * (H // G)
    nh = 2 * G
    gw = G * DH
    wo_rows = gw // B
    wq_rows = D // B // WQ_SPLIT
    x_rows = KV_ROWS * DH // D
    w_lead = B + Q_AHEAD - 1
    qscale = DH**-0.5 * math.log2(math.e)
    orders = _kv_orders(SK)
    npair = len(orders[0])
    assert B == 1 << log_b and H % G == 0 and w_lead + 2 <= nstep and 2 <= Q_AHEAD <= B
    assert LEAD[0] <= LEAD[1] <= npair and SQ % OUT_ROWS == 0 and B * SQ % x_rows == 0

    def kernel(
        ax, ak, av, awq, awo, bx, bk, bv, bwq, bwo, out,
        xs, wq, wo, kv, acc, ob, q_ring, p_carry, r_carry, o_carry,
        first_sem, kv_sem, w_sem, out_sem,
    ):
        caches = (ak, av, bk, bv)
        copy = pltpu.make_async_copy

        def kv_copy(i, m, prio):
            cache, row = orders[prio][m]
            base = ((i & (B - 1)) * H + (i >> log_b) * G) * SK
            slot = i & (NSLOT - 1)
            return copy(
                caches[cache].at[pl.ds(pl.multiple_of(base + row, KV_ROWS), KV_ROWS)],
                kv.at[slot, cache, pl.ds(row, KV_ROWS)],
                kv_sem.at[slot],
            )

        def kv_issue(i, lo, hi, near_end=False):
            for m in range(lo, hi):
                for prio in range(2):
                    ahead, u = divmod(m + LEAD[prio], npair)
                    target = i + 1 + ahead

                    def start():
                        kv_copy(target, u, prio).start(priority=prio)

                    if near_end:
                        pl.when(target < nstep)(start)
                    else:
                        start()

        def kv_wait(i):
            slot = i & (NSLOT - 1)
            copy(kv.at[slot], kv.at[slot], kv_sem.at[slot]).wait()

        def w_copies(w, sem):
            col = pl.multiple_of((w >> log_b) * gw, gw)
            rq = pl.ds(pl.multiple_of((w & (B - 1)) * wq_rows, wq_rows), wq_rows)
            ro = pl.ds(pl.multiple_of(col + (w & (B - 1)) * wo_rows, wo_rows), wo_rows)
            cols = pl.ds(col, gw)
            return [
                copy(awq.at[:, rq, cols], wq.at[0, :, rq, cols], sem),
                copy(awo.at[ro], wo.at[0, ro], sem),
                copy(bwq.at[:, rq, cols], wq.at[1, :, rq, cols], sem),
                copy(bwo.at[ro], wo.at[1, ro], sem),
            ]

        def w_issue(i):
            copies = w_copies(i + w_lead, w_sem.at[i & (NSLOT - 1)])
            for n, cp in enumerate(copies):
                cp.start(priority=n % 2)

        def out_issue(b0, nb):
            for row in range(0, SQ, OUT_ROWS):
                part = (pl.ds(b0, nb), pl.ds(row, OUT_ROWS))
                copy(ob.at[part], out.at[part], out_sem.at[0]).start()

        def run(i, items, hook=None):
            probs, outs = {}, {}
            for t, (stage, n) in enumerate(items):
                if hook is not None:
                    hook(t)
                step = i + (Q_AHEAD if stage == "qp" else n // nh)
                slot = step & (NSLOT - 1)
                if n < 0:
                    step = jnp.maximum(step, 0)
                b = step & (B - 1)
                br, h = divmod(n % nh, G)
                head = pl.ds(pl.multiple_of(((step >> log_b) * G + h) * DH, DH), DH)
                keys = pl.ds(h * SK, SK)
                if stage == "qp":
                    x = xs[br, pl.ds(pl.multiple_of(b * SQ, SQ), SQ)]
                    w = [wq[br, u, :, head] for u in range(WQ_SPLIT)]
                    w = jnp.concatenate(w, axis=0)
                    q = jnp.dot(x, w, preferred_element_type=f32)
                    q_ring[i & (Q_AHEAD - 1), n] = (q * qscale).astype(bf16)
                elif stage == "qk":
                    q = q_ring[i & (Q_AHEAD - 1), n]
                    k = kv[slot, 2 * br, keys]
                    s = lax.dot_general(q, k, _NT, preferred_element_type=f32)
                    p, r = [], []
                    for m in range(0, SQ, SOFTMAX_ROWS):
                        sm = s[m : m + SOFTMAX_ROWS]
                        e = jnp.exp2(sm - jnp.max(sm, axis=-1, keepdims=True))
                        r.append(1.0 / jnp.sum(e, axis=-1, keepdims=True))
                        p.append(e.astype(bf16))
                    p, r = jnp.concatenate(p, axis=0), jnp.concatenate(r, axis=0)
                    if ("pv", n) in items:
                        probs[n] = (p, r)
                    else:
                        p_carry[...] = p
                        r_carry[...] = jnp.broadcast_to(r, (SQ, DH))
                elif stage == "pv":
                    p, r = probs.pop(n) if n in probs else (p_carry[...], r_carry[...])
                    v = kv[slot, 2 * br + 1, keys]
                    o = (jnp.dot(p, v, preferred_element_type=f32) * r).astype(bf16)
                    if ("op", n) in items:
                        outs[n] = o
                    else:
                        o_carry[n % 2] = o
                else:
                    o = outs.pop(n) if n in outs else o_carry[n % 2]
                    if n < 0:
                        b = jnp.where(i == 0, B, b)
                    w = wo[br, head, :]
                    a = acc[b, br] + jnp.dot(o, w, preferred_element_type=f32)
                    acc[b, br] = a
                    if h == G - 1:
                        ob[b, :, br * D : (br + 1) * D] = a.astype(bf16)

        first = []
        for c in _scattered_pairs(B * SQ // x_rows):
            part = pl.ds(c * x_rows, x_rows)
            first.append(copy(ax.at[part], xs.at[0, part], first_sem.at[0]))
            first.append(copy(bx.at[part], xs.at[1, part], first_sem.at[0]))
        for w in range(w_lead):
            first += w_copies(w, first_sem.at[0])
        queues = [
            first[prio::2] + [kv_copy(0, m, prio) for m in range(LEAD[prio])]
            for prio in range(2)
        ]
        skew = LEAD[1] - LEAD[0]
        for cp in queues[1][:skew]:
            cp.start(priority=1)
        pairs = list(zip(queues[0], queues[1][skew:]))
        for part in range(3):
            lo, hi = part * len(pairs) // 3, (part + 1) * len(pairs) // 3
            for cp0, cp1 in pairs[lo:hi]:
                cp0.start(priority=0)
                cp1.start(priority=1)

            @pl.loop(part * (B + 1) // 3, (part + 1) * (B + 1) // 3)
            def _(b):
                acc[b] = jnp.zeros((2, SQ, D), f32)

        w_issue(0)
        w_issue(1)
        o_carry[...] = jnp.zeros_like(o_carry)
        p_carry[...] = jnp.zeros_like(p_carry)
        r_carry[...] = jnp.zeros_like(r_carry)
        kv[NSLOT - 1, 3, pl.ds((G - 1) * SK, SK)] = jnp.zeros((SK, DH), bf16)
        for cp in first:
            cp.wait()

        @pl.loop(0, Q_AHEAD)
        def _(k):
            for u in range(Q_AHEAD):

                @pl.when(k == u)
                def _():
                    kv_issue(-1, u * npair // Q_AHEAD, (u + 1) * npair // Q_AHEAD)

            run(k - Q_AHEAD, [("qp", n) for n in range(nh)])

        def spread(i, t, n, near_end=False):
            if t > 0:
                lo = 0 if t == 1 else t * npair // n
                kv_issue(i, lo, (t + 1) * npair // n, near_end)

        @pl.loop(0, nstep - Q_AHEAD)
        def _(i):
            kv_wait(i)

            @pl.when(i + w_lead < nstep)
            def _():
                for cp in w_copies(i + w_lead, w_sem.at[i & (NSLOT - 1)]):
                    cp.wait()

            def hook(t):
                if t == len(STEP_ITEMS) // 2:
                    pl.when(i + 2 + w_lead < nstep)(lambda: w_issue(i + 2))
                spread(i, t, len(STEP_ITEMS))

            run(i, STEP_ITEMS, hook)

        @pl.loop(nstep - Q_AHEAD, nstep)
        def _(i):
            pl.when(i == nstep - 1)(lambda: out_issue(0, B - 2))
            kv_wait(i)
            items = [item for item in STEP_ITEMS if item[0] != "qp"]
            run(i, items, lambda t: spread(i, t, len(items), near_end=True))

        run(nstep, DRAIN_ITEMS)
        out_issue(B - 2, 2)
        copy(ob.at[pl.ds(0, B)], out, out_sem.at[0]).wait()

    dma_sem = pltpu.SemaphoreType.DMA
    scratch = [
        pltpu.VMEM((2, B * SQ, D), bf16),
        pltpu.VMEM((2, WQ_SPLIT, D // WQ_SPLIT, H * DH), bf16),
        pltpu.VMEM((2, H * DH, D), bf16),
        pltpu.VMEM((NSLOT, 4, G * SK, DH), bf16),
        pltpu.VMEM((B + 1, 2, SQ, D), f32),
        pltpu.VMEM((B + 1, SQ, 2 * D), bf16),
        pltpu.VMEM((Q_AHEAD, nh, SQ, DH), bf16),
        pltpu.VMEM((SQ, SK), bf16),
        pltpu.VMEM((SQ, DH), f32),
        pltpu.VMEM((2, SQ, DH), bf16),
        dma_sem((1,)),
        dma_sem((NSLOT,)),
        dma_sem((NSLOT,)),
        dma_sem((1,)),
    ]
    return kernel, scratch


@jax.jit
def pallas_concat_heads__mha_block_cached__gqa_block_cached__near_ridge_kernel(
    A_x: jax.Array,
    A_k_cache: jax.Array,
    A_v_cache: jax.Array,
    A_wq: jax.Array,
    A_wo: jax.Array,
    B_x: jax.Array,
    B_k_cache: jax.Array,
    B_v_cache: jax.Array,
    B_wq: jax.Array,
    B_wo: jax.Array,
):
    B, SQ, D = A_x.shape
    _, H, SK, dh = A_k_cache.shape
    assert dh == DH and B_x.shape == A_x.shape and B_k_cache.shape == A_k_cache.shape
    kernel, scratch = _make_kernel(B, SQ, D, H, SK)

    def rows(t):
        return t.reshape(-1, t.shape[-1])

    def split(w):
        return w.reshape(WQ_SPLIT, D // WQ_SPLIT, H * DH)

    return pl.pallas_call(
        kernel,
        in_specs=[pl.BlockSpec(memory_space=pl.ANY)] * 10,
        out_specs=pl.BlockSpec(memory_space=pl.ANY),
        out_shape=jax.ShapeDtypeStruct((B, SQ, 2 * D), A_x.dtype),
        scratch_shapes=scratch,
        compiler_params=pltpu.CompilerParams(
            vmem_limit_bytes=100 * 1024 * 1024, disable_bounds_checks=True
        ),
    )(
        rows(A_x), rows(A_k_cache), rows(A_v_cache), split(A_wq), A_wo,
        rows(B_x), rows(B_k_cache), rows(B_v_cache), split(B_wq), B_wo,
    )
```

```python
import math

import jax
import jax.numpy as jnp
from jax import lax
import jax.experimental.pallas as pl
import jax.experimental.pallas.tpu as pltpu

DH = 128
G = 4
NSLOT = 4
KV_ROWS = 128
LEAD = (22, 48)
Q_AHEAD = 4
WQ_SPLIT = 4
OUT_ROWS = 8
OUT_OVERLAP = 10
SOFTMAX_ROWS = 16

STEP_ITEMS = (
    ("pv", -1), ("op", -3), ("op", -2), ("qk", 0), ("qp", 0), ("qk", 1), ("qp", 1), ("pv", 0),
    ("qk", 2), ("qp", 2), ("pv", 1), ("op", -1), ("op", 0), ("qk", 3), ("qp", 3), ("pv", 2),
    ("qk", 4), ("op", 1), ("qp", 4), ("op", 2), ("pv", 3), ("qk", 5), ("qp", 5), ("pv", 4),
    ("op", 3), ("qk", 6), ("qp", 6), ("qk", 7), ("pv", 5), ("op", 4), ("qp", 7), ("pv", 6),
)
DRAIN_ITEMS = (("pv", -1), ("op", -3), ("op", -2), ("op", -1))
_NT = (((1,), (1,)), ((), ()))


def _scattered_pairs(n):
    npairs = n // 2
    assert n % 2 == 0 and math.gcd(9, npairs) == 1
    return [(2 * (9 * k % npairs) + 1 + u) % n for k in range(npairs) for u in range(2)]


def _kv_orders(sk):
    nchunk = G * sk // KV_ROWS
    nblock = 2 * nchunk
    assert math.gcd(9, nblock) == 1
    orders = ([], [])
    for k in range(nblock):
        pair, cache = divmod(9 * k % nblock, 4)
        for u in range(2):
            orders[k % 2].append((cache, (2 * pair + 1 + u) % nchunk * KV_ROWS))
    shift = LEAD[1] - LEAD[0]
    return orders[0][shift:] + orders[0][:shift], orders[1]


def _make_kernel(B, SQ, D, H, SK):
    bf16, f32 = jnp.bfloat16, jnp.float32
    log_b = B.bit_length() - 1
    nstep = B * (H // G)
    nh = 2 * G
    gw = G * DH
    wo_rows = gw // B
    wq_rows = D // B // WQ_SPLIT
    x_rows = KV_ROWS * DH // D
    w_lead = B + Q_AHEAD - 1
    qscale = DH**-0.5 * math.log2(math.e)
    orders = _kv_orders(SK)
    npair = len(orders[0])
    assert B == 1 << log_b and H % G == 0 and w_lead + 2 <= nstep and 2 <= Q_AHEAD <= B
    assert LEAD[0] <= LEAD[1] <= npair and SQ % OUT_ROWS == 0 and B * SQ % x_rows == 0

    def kernel(
        ax, ak, av, awq, awo, bx, bk, bv, bwq, bwo, out,
        xs, wq, wo, kv, acc, ob, q_ring, p_carry, r_carry, o_carry,
        first_sem, kv_sem, w_sem, out_sem,
    ):
        caches = (ak, av, bk, bv)
        copy = pltpu.make_async_copy

        def kv_copy(i, m, prio):
            cache, row = orders[prio][m]
            base = ((i & (B - 1)) * H + (i >> log_b) * G) * SK
            slot = i & (NSLOT - 1)
            return copy(
                caches[cache].at[pl.ds(pl.multiple_of(base + row, KV_ROWS), KV_ROWS)],
                kv.at[slot, cache, pl.ds(row, KV_ROWS)],
                kv_sem.at[slot],
            )

        def kv_issue(i, lo, hi, near_end=False):
            for m in range(lo, hi):
                for prio in range(2):
                    ahead, u = divmod(m + LEAD[prio], npair)
                    target = i + 1 + ahead

                    def start():
                        kv_copy(target, u, prio).start(priority=prio)

                    if near_end:
                        pl.when(target < nstep)(start)
                    else:
                        start()

        def kv_wait(i):
            slot = i & (NSLOT - 1)
            copy(kv.at[slot], kv.at[slot], kv_sem.at[slot]).wait()

        def w_copies(w, sem):
            col = pl.multiple_of((w >> log_b) * gw, gw)
            rq = pl.ds(pl.multiple_of((w & (B - 1)) * wq_rows, wq_rows), wq_rows)
            ro = pl.ds(pl.multiple_of(col + (w & (B - 1)) * wo_rows, wo_rows), wo_rows)
            cols = pl.ds(col, gw)
            return [
                copy(awq.at[:, rq, cols], wq.at[0, :, rq, cols], sem),
                copy(awo.at[ro], wo.at[0, ro], sem),
                copy(bwq.at[:, rq, cols], wq.at[1, :, rq, cols], sem),
                copy(bwo.at[ro], wo.at[1, ro], sem),
            ]

        def w_issue(i):
            copies = w_copies(i + w_lead, w_sem.at[i & (NSLOT - 1)])
            for n, cp in enumerate(copies):
                cp.start(priority=n % 2)

        def out_issue(b0, nb):
            for row in range(0, SQ, OUT_ROWS):
                part = (pl.ds(b0, nb), pl.ds(row, OUT_ROWS))
                copy(ob.at[part], out.at[part], out_sem.at[0]).start()

        def run(i, items, hook=None):
            probs, outs = {}, {}
            for t, (stage, n) in enumerate(items):
                if hook is not None:
                    hook(t)
                step = i + (Q_AHEAD if stage == "qp" else n // nh)
                slot = step & (NSLOT - 1)
                if n < 0:
                    step = jnp.maximum(step, 0)
                b = step & (B - 1)
                br, h = divmod(n % nh, G)
                head = pl.ds(pl.multiple_of(((step >> log_b) * G + h) * DH, DH), DH)
                keys = pl.ds(h * SK, SK)
                if stage == "qp":
                    x = xs[br, pl.ds(pl.multiple_of(b * SQ, SQ), SQ)]
                    w = [wq[br, u, :, head] for u in range(WQ_SPLIT)]
                    w = jnp.concatenate(w, axis=0)
                    q = jnp.dot(x, w, preferred_element_type=f32)
                    q_ring[i & (Q_AHEAD - 1), n] = (q * qscale).astype(bf16)
                elif stage == "qk":
                    q = q_ring[i & (Q_AHEAD - 1), n]
                    k = kv[slot, 2 * br, keys]
                    s = lax.dot_general(q, k, _NT, preferred_element_type=f32)
                    p, r = [], []
                    for m in range(0, SQ, SOFTMAX_ROWS):
                        sm = s[m : m + SOFTMAX_ROWS]
                        e = jnp.exp2(sm - jnp.max(sm, axis=-1, keepdims=True))
                        r.append(1.0 / jnp.sum(e, axis=-1, keepdims=True))
                        p.append(e.astype(bf16))
                    p, r = jnp.concatenate(p, axis=0), jnp.concatenate(r, axis=0)
                    if ("pv", n) in items:
                        probs[n] = (p, r)
                    else:
                        p_carry[...] = p
                        r_carry[...] = jnp.broadcast_to(r, (SQ, DH))
                elif stage == "pv":
                    p, r = probs.pop(n) if n in probs else (p_carry[...], r_carry[...])
                    v = kv[slot, 2 * br + 1, keys]
                    o = (jnp.dot(p, v, preferred_element_type=f32) * r).astype(bf16)
                    if ("op", n) in items:
                        outs[n] = o
                    else:
                        o_carry[n % 2] = o
                else:
                    o = outs.pop(n) if n in outs else o_carry[n % 2]
                    if n < 0:
                        b = jnp.where(i == 0, B, b)
                    w = wo[br, head, :]
                    a = acc[b, br] + jnp.dot(o, w, preferred_element_type=f32)
                    acc[b, br] = a
                    if h == G - 1:
                        ob[b, :, br * D : (br + 1) * D] = a.astype(bf16)

        first = []
        for c in _scattered_pairs(B * SQ // x_rows):
            part = pl.ds(c * x_rows, x_rows)
            first.append(copy(ax.at[part], xs.at[0, part], first_sem.at[0]))
            first.append(copy(bx.at[part], xs.at[1, part], first_sem.at[0]))
        for w in range(w_lead):
            first += w_copies(w, first_sem.at[0])
        queues = [
            first[prio::2] + [kv_copy(0, m, prio) for m in range(LEAD[prio])]
            for prio in range(2)
        ]
        skew = LEAD[1] - LEAD[0]
        for cp in queues[1][:skew]:
            cp.start(priority=1)
        pairs = list(zip(queues[0], queues[1][skew:]))
        for part in range(3):
            lo, hi = part * len(pairs) // 3, (part + 1) * len(pairs) // 3
            for cp0, cp1 in pairs[lo:hi]:
                cp0.start(priority=0)
                cp1.start(priority=1)

            @pl.loop(part * (B + 1) // 3, (part + 1) * (B + 1) // 3)
            def _(b):
                acc[b] = jnp.zeros((2, SQ, D), f32)

        w_issue(0)
        w_issue(1)
        o_carry[...] = jnp.zeros_like(o_carry)
        p_carry[...] = jnp.zeros_like(p_carry)
        r_carry[...] = jnp.zeros_like(r_carry)
        kv[NSLOT - 1, 3, pl.ds((G - 1) * SK, SK)] = jnp.zeros((SK, DH), bf16)
        for cp in first:
            cp.wait()

        @pl.loop(0, Q_AHEAD)
        def _(k):
            for u in range(Q_AHEAD):

                @pl.when(k == u)
                def _():
                    kv_issue(-1, u * npair // Q_AHEAD, (u + 1) * npair // Q_AHEAD)

            run(k - Q_AHEAD, [("qp", n) for n in range(nh)])

        def spread(i, t, n, near_end=False):
            if t > 0:
                lo = 0 if t == 1 else t * npair // n
                kv_issue(i, lo, (t + 1) * npair // n, near_end)

        @pl.loop(0, nstep - Q_AHEAD)
        def _(i):
            kv_wait(i)

            @pl.when(i + w_lead < nstep)
            def _():
                for cp in w_copies(i + w_lead, w_sem.at[i & (NSLOT - 1)]):
                    cp.wait()

            def hook(t):
                if t == len(STEP_ITEMS) // 2:
                    pl.when(i + 2 + w_lead < nstep)(lambda: w_issue(i + 2))
                spread(i, t, len(STEP_ITEMS))

            run(i, STEP_ITEMS, hook)

        @pl.loop(nstep - Q_AHEAD, nstep)
        def _(i):
            copies = [kv_copy(i, m, prio) for m in range(npair) for prio in range(2)]
            for cp in copies[:-OUT_OVERLAP]:
                cp.wait()
            pl.when(i == nstep - 1)(lambda: out_issue(0, B - 2))
            for cp in copies[-OUT_OVERLAP:]:
                cp.wait()
            items = [item for item in STEP_ITEMS if item[0] != "qp"]
            run(i, items, lambda t: spread(i, t, len(items), near_end=True))

        run(nstep, DRAIN_ITEMS)
        out_issue(B - 2, 2)
        copy(ob.at[pl.ds(0, B)], out, out_sem.at[0]).wait()

    dma_sem = pltpu.SemaphoreType.DMA
    scratch = [
        pltpu.VMEM((2, B * SQ, D), bf16),
        pltpu.VMEM((2, WQ_SPLIT, D // WQ_SPLIT, H * DH), bf16),
        pltpu.VMEM((2, H * DH, D), bf16),
        pltpu.VMEM((NSLOT, 4, G * SK, DH), bf16),
        pltpu.VMEM((B + 1, 2, SQ, D), f32),
        pltpu.VMEM((B + 1, SQ, 2 * D), bf16),
        pltpu.VMEM((Q_AHEAD, nh, SQ, DH), bf16),
        pltpu.VMEM((SQ, SK), bf16),
        pltpu.VMEM((SQ, DH), f32),
        pltpu.VMEM((2, SQ, DH), bf16),
        dma_sem((1,)),
        dma_sem((NSLOT,)),
        dma_sem((NSLOT,)),
        dma_sem((1,)),
    ]
    return kernel, scratch


@jax.jit
def pallas_concat_heads__mha_block_cached__gqa_block_cached__near_ridge_kernel(
    A_x: jax.Array,
    A_k_cache: jax.Array,
    A_v_cache: jax.Array,
    A_wq: jax.Array,
    A_wo: jax.Array,
    B_x: jax.Array,
    B_k_cache: jax.Array,
    B_v_cache: jax.Array,
    B_wq: jax.Array,
    B_wo: jax.Array,
):
    B, SQ, D = A_x.shape
    _, H, SK, dh = A_k_cache.shape
    assert dh == DH and B_x.shape == A_x.shape and B_k_cache.shape == A_k_cache.shape
    kernel, scratch = _make_kernel(B, SQ, D, H, SK)

    def rows(t):
        return t.reshape(-1, t.shape[-1])

    def split(w):
        return w.reshape(WQ_SPLIT, D // WQ_SPLIT, H * DH)

    return pl.pallas_call(
        kernel,
        in_specs=[pl.BlockSpec(memory_space=pl.ANY)] * 10,
        out_specs=pl.BlockSpec(memory_space=pl.ANY),
        out_shape=jax.ShapeDtypeStruct((B, SQ, 2 * D), A_x.dtype),
        scratch_shapes=scratch,
        compiler_params=pltpu.CompilerParams(
            vmem_limit_bytes=100 * 1024 * 1024, disable_bounds_checks=True
        ),
    )(
        rows(A_x), rows(A_k_cache), rows(A_v_cache), split(A_wq), A_wo,
        rows(B_x), rows(B_k_cache), rows(B_v_cache), split(B_wq), B_wo,
    )
```
